```python
import os as _os
_os.environ.setdefault("JAX_PLATFORMS", "cpu")
import jax
import jax.numpy as jnp

def _softmax(x, axis=-1):
    return jax.nn.softmax(x, axis=axis)
def _gelu(x):
    return jax.nn.gelu(x, approximate=True)
def _silu(x):
    return jax.nn.silu(x)
def _sigmoid(x):
    return jax.nn.sigmoid(x)
def _layernorm(x, axis=-1, eps=1e-5):
    m = jnp.mean(x, axis=axis, keepdims=True)
    v = jnp.var(x, axis=axis, keepdims=True)
    return (x - m) / jnp.sqrt(v + eps)
def _scatter_add(tgt, idx, src, axis=0):
    return tgt.at[idx].add(src)
def _segment_sum(src, seg, n):
    return jax.ops.segment_sum(src, seg, n)
class _Rng:
    def __init__(self, key):
        self._k = key
    def _next(self):
        self._k, sub = jax.random.split(self._k)
        return sub
    def normal(self, shape):
        return jax.random.normal(self._next(), shape, dtype=jnp.bfloat16)
    def randint(self, lo, hi, shape):
        return jax.random.randint(self._next(), shape, lo, hi, dtype=jnp.int32)
    def uniform(self, shape, lo=0.0, hi=1.0):
        return jax.random.uniform(self._next(), shape, jnp.bfloat16, lo, hi)
    def permutation(self, n):
        return jax.random.permutation(self._next(), n)


kernel_name = 'standalone__gqa_softmax__near_ridge'

def setup_inputs():
    _rng = _Rng(jax.random.key(int.from_bytes(__import__("os").urandom(4), "little")))
    _w = (lambda a: (lambda t: t.astype(jnp.bfloat16) if jnp.issubdtype(t.dtype, jnp.floating) else t)(jnp.asarray(a)))
    B, Hq, Hkv, Sq, Sk, D = 8, 16, 8, 160, 2048, 256
    return {
        "q": _w((lambda *s: _rng.normal(s) * 0.05)(B, Hq, Sq, D)),
        "k": _w((lambda *s: _rng.normal(s) * 3.2)(B, Hkv, Sk, D)),
        "v": _w((lambda *s: _rng.normal(s) * 0.05)(B, Hkv, Sk, D)),
    }

def reference(q, k, v):
    B, Hq, Sq, D = q.shape
    Hkv = k.shape[1]
    rep = Hq // Hkv
    k = jnp.repeat(k, rep, axis=1)
    v = jnp.repeat(v, rep, axis=1)
    scale = D ** -0.5
    scores = jnp.einsum("bhqd,bhkd->bhqk", q, k) * scale
    p = _softmax(scores, axis=-1)
    return jnp.einsum("bhqk,bhkd->bhqd", p, v)
```

```python
import jax
import jax.numpy as jnp
import jax.experimental.pallas as pl
import jax.experimental.pallas.tpu as pltpu

CK = 256
LEAD = 1
HPS = 2

@jax.jit
def pallas_standalone__gqa_softmax__near_ridge_kernel(q, k, v):
    B, Hq, Sq, D = q.shape
    Hkv, Sk = k.shape[1], k.shape[2]
    rep = Hq // Hkv
    M = rep * Sq
    scale = D ** -0.5
    G = B * Hkv
    NS = G // HPS
    q3 = q.reshape(G, M, D)
    k3 = k.reshape(G, Sk, D)
    v3 = v.reshape(G, Sk, D)
    NC = Sk // CK
    NT = CK // 128

    def kernel(q_ref, k_ref, v_ref, o_ref, *scr):
        i = pl.program_id(0)
        bufs = [scr[0:4], scr[4:8]]

        def body(par, do1, do2, do3):
            sw_ref, mw_ref = bufs[par][0], bufs[par][1]
            sr_ref, mr_ref = bufs[1 - par][0], bufs[1 - par][1]
            ow_ref, lw_ref = bufs[par][2], bufs[par][3]
            or_ref, lr_ref = bufs[1 - par][2], bufs[1 - par][3]
            mstate = [None] * HPS

            def qk(t):
                h, c = divmod(t, NC)
                s = jax.lax.dot_general(q_ref[h], k_ref[h, c * CK:(c + 1) * CK, :], (((1,), (1,)), ((), ())),
                                        preferred_element_type=jnp.float32)
                sw_ref[h, :, c * CK:(c + 1) * CK] = s
                for j in range(NT):
                    sj = s[:, j * 128:(j + 1) * 128]
                    mstate[h] = sj if mstate[h] is None else jnp.maximum(mstate[h], sj)
                if c == NC - 1:
                    m = jnp.max(mstate[h], axis=-1, keepdims=True)
                    mw_ref[h] = jnp.broadcast_to(m, (M, 128))

            if do3:
                for h in range(HPS):
                    l = jnp.sum(lr_ref[h], axis=-1, keepdims=True)
                    o_ref[h] = (or_ref[h] * (1.0 / l)).astype(o_ref.dtype)
            T = HPS * NC
            if do1 and not do2:
                for t in range(T):
                    qk(t)
                return
            if not do2:
                return
            if do1:
                for t in range(LEAD):
                    qk(t)
            for h in range(HPS):
                l_run = None
                o = None
                for c in range(NC):
                    mm = mr_ref[h]
                    p = jnp.exp((sr_ref[h, :, c * CK:(c + 1) * CK] - jnp.concatenate([mm] * NT, axis=1)) * scale)
                    for j in range(NT):
                        pj = p[:, j * 128:(j + 1) * 128]
                        l_run = pj if l_run is None else l_run + pj
                    oc = jnp.dot(p.astype(jnp.bfloat16), v_ref[h, c * CK:(c + 1) * CK, :],
                                 preferred_element_type=jnp.float32)
                    o = oc if o is None else o + oc
                    t = h * NC + c + LEAD
                    if do1 and t < T:
                        qk(t)
                ow_ref[h] = o
                lw_ref[h] = l_run

        @pl.when(i == 0)
        def _():
            body(0, True, False, False)

        @pl.when(i == 1)
        def _():
            body(1, True, True, False)

        @pl.when(jnp.logical_and(jnp.logical_and(i > 1, i < NS), i % 2 == 0))
        def _():
            body(0, True, True, True)

        @pl.when(jnp.logical_and(jnp.logical_and(i > 1, i < NS), i % 2 == 1))
        def _():
            body(1, True, True, True)

        @pl.when(i == NS)
        def _():
            body(NS % 2, False, True, True)

        @pl.when(i == NS + 1)
        def _():
            body((NS + 1) % 2, False, False, True)

    one = [pltpu.VMEM((HPS, M, Sk), jnp.float32), pltpu.VMEM((HPS, M, 128), jnp.float32),
           pltpu.VMEM((HPS, M, D), jnp.float32), pltpu.VMEM((HPS, M, 128), jnp.float32)]
    out = pl.pallas_call(
        kernel,
        grid=(NS + 2,),
        in_specs=[
            pl.BlockSpec((HPS, M, D), lambda i: (jnp.minimum(i, NS - 1), 0, 0)),
            pl.BlockSpec((HPS, Sk, D), lambda i: (jnp.minimum(i, NS - 1), 0, 0)),
            pl.BlockSpec((HPS, Sk, D), lambda i: (jnp.clip(i - 1, 0, NS - 1), 0, 0)),
        ],
        out_specs=pl.BlockSpec((HPS, M, D), lambda i: (jnp.maximum(i - 2, 0), 0, 0)),
        out_shape=jax.ShapeDtypeStruct((G, M, D), q.dtype),
        scratch_shapes=one + one,
        compiler_params=pltpu.CompilerParams(
            dimension_semantics=("arbitrary",),
            vmem_limit_bytes=100 * 1024 * 1024,
        ),
    )(q3, k3, v3)
    return out.reshape(B, Hq, Sq, D)
```

```python
import jax
import jax.numpy as jnp
import jax.experimental.pallas as pl
import jax.experimental.pallas.tpu as pltpu

CK = 256
LEAD = 1
NF = 2


@jax.jit
def pallas_standalone__gqa_softmax__near_ridge_kernel(
    q: jax.Array,
    k: jax.Array,
    v: jax.Array,
):
    B, Hq, Sq, D = q.shape
    Hkv, Sk = k.shape[1], k.shape[2]
    rep = Hq // Hkv
    M = rep * Sq
    scale = D ** -0.5
    G = B * Hkv
    q3 = q.reshape(G, M, D)
    k3 = k.reshape(G, Sk, D)
    v3 = v.reshape(G, Sk, D)
    NC = Sk // CK
    NT = CK // 128
    NR = 4 + 4 * NF
    J0 = NR // 2
    NP = G // 2
    assert G % 4 == 0 and G >= NR + 4 and Sk % CK == 0 and CK % 128 == 0

    def kernel(q_hbm, k_hbm, v_hbm, o_hbm, qbuf, kbuf, vbuf, obuf, s_ref, m_ref, ou_ref, l_ref,
               qsem, ksem, vsem, osem):

        def qcopy(h, sl):
            return pltpu.make_async_copy(q_hbm.at[h], qbuf.at[sl], qsem.at[sl])

        def kcopy(h, sl):
            return pltpu.make_async_copy(k_hbm.at[h], kbuf.at[sl], ksem.at[sl])

        def vcopy(h, sl):
            return pltpu.make_async_copy(v_hbm.at[h], vbuf.at[sl], vsem.at[sl])

        def ocopy(h, sl):
            return pltpu.make_async_copy(obuf.at[sl], o_hbm.at[h], osem.at[sl])

        def start_qk(h, sl):
            qcopy(h, sl).start()
            kcopy(h, sl).start()

        def wait_qk(h, sl):
            qcopy(h, sl).wait()
            kcopy(h, sl).wait()

        def compute(As, Bs, Fs):
            mstate = {}

            def qk(t):
                a, c = divmod(t, NC)
                sl = As[a]
                s = jax.lax.dot_general(qbuf[sl], kbuf[sl, c * CK:(c + 1) * CK, :],
                                        (((1,), (1,)), ((), ())),
                                        preferred_element_type=jnp.float32)
                s_ref[sl, :, c * CK:(c + 1) * CK] = s
                for j in range(NT):
                    sj = s[:, j * 128:(j + 1) * 128]
                    mstate[sl] = sj if sl not in mstate else jnp.maximum(mstate[sl], sj)
                if c == NC - 1:
                    m = jnp.max(mstate[sl], axis=-1, keepdims=True)
                    m_ref[sl] = jnp.broadcast_to(m, (M, 128))

            for sl in Fs:
                l = jnp.sum(l_ref[sl], axis=-1, keepdims=True)
                r = pl.reciprocal(l, approx=True)
                r = r * (2.0 - l * r)
                obuf[sl] = (ou_ref[sl] * r).astype(obuf.dtype)

            T = len(As) * NC
            done = 0
            if Bs:
                for t in range(min(LEAD, T)):
                    qk(t)
                    done += 1
            for sl in Bs:
                l_run = None
                o = None
                for c in range(NC):
                    mm = m_ref[sl]
                    p = jnp.exp((s_ref[sl, :, c * CK:(c + 1) * CK]
                                 - jnp.concatenate([mm] * NT, axis=1)) * scale)
                    for j in range(NT):
                        pj = p[:, j * 128:(j + 1) * 128]
                        l_run = pj if l_run is None else l_run + pj
                    oc = jnp.dot(p.astype(vbuf.dtype), vbuf[sl, c * CK:(c + 1) * CK, :],
                                 preferred_element_type=jnp.float32)
                    o = oc if o is None else o + oc
                    if done < T:
                        qk(done)
                        done += 1
                ou_ref[sl] = o
                l_ref[sl] = l_run
            while done < T:
                qk(done)
                done += 1

        start_qk(0, 0)
        start_qk(1, 1)
        start_qk(2, 2)
        vcopy(0, 0).start()
        start_qk(3, 3)
        vcopy(1, 1).start()
        for r in range(4):
            wait_qk(r, r)
            if r >= 2:
                vcopy(r - 2, r - 2).wait()
            compute([r], [r - 2] if r >= 2 else [], [])
            start_qk(r + 4, r)
            vcopy(r + 2, (r + 2) % 4).start()

        def fine_body(t, carry):
            for u in range(4):
                h = 4 + 4 * t + u
                wait_qk(h, u)
                vcopy(h - 2, (u + 2) % 4).wait()

                @pl.when(t >= 1)
                def _():
                    ocopy(h - 8, u).wait()
                compute([u], [(u + 2) % 4], [u])
                ocopy(h - 4, u).start()
                start_qk(h + 4, u)
                vcopy(h + 2, (u + 2) % 4).start()
            return carry
        jax.lax.fori_loop(0, NF, fine_body, 0)

        def block(j, par):
            sA = [2 * par, 2 * par + 1]
            sB = [2 * (1 - par), 2 * (1 - par) + 1]
            for a in range(2):
                wait_qk(2 * j + a, sA[a])
                vcopy(2 * j - 2 + a, sB[a]).wait()
            for a in range(2):
                ocopy(2 * j - 8 + a, sA[a]).wait()
            compute(sA, sB, sA)
            for a in range(2):
                ocopy(2 * j - 4 + a, sA[a]).start()

            @pl.when(j + 2 < NP)
            def _():
                start_qk(2 * j + 4, sA[0])

            @pl.when(j + 1 < NP)
            def _():
                vcopy(2 * j + 2, sB[0]).start()

            @pl.when(j + 2 < NP)
            def _():
                start_qk(2 * j + 5, sA[1])

            @pl.when(j + 1 < NP)
            def _():
                vcopy(2 * j + 3, sB[1]).start()

        def loop_body(t, carry):
            jj = J0 + 2 * t
            block(jj, 0)
            block(jj + 1, 1)
            return carry
        jax.lax.fori_loop(0, (NP - J0) // 2, loop_body, 0)

        hB = [G - 2, G - 1]
        hF = [G - 4, G - 3]
        for h in hB:
            vcopy(h, h % 4).wait()
        for h in hF:
            ocopy(h - 4, h % 4).wait()
        compute([], [h % 4 for h in hB], [h % 4 for h in hF])
        for h in hF:
            ocopy(h, h % 4).start()
        hF = [G - 2, G - 1]
        for h in hF:
            ocopy(h - 4, h % 4).wait()
        compute([], [], [h % 4 for h in hF])
        for h in hF:
            ocopy(h, h % 4).start()
        for h in range(G - 4, G):
            ocopy(h, h % 4).wait()

    out = pl.pallas_call(
        kernel,
        in_specs=[pl.BlockSpec(memory_space=pl.ANY)] * 3,
        out_specs=pl.BlockSpec(memory_space=pl.ANY),
        out_shape=jax.ShapeDtypeStruct((G, M, D), q.dtype),
        scratch_shapes=[
            pltpu.VMEM((4, M, D), q.dtype),
            pltpu.VMEM((4, Sk, D), k.dtype),
            pltpu.VMEM((4, Sk, D), v.dtype),
            pltpu.VMEM((4, M, D), q.dtype),
            pltpu.VMEM((4, M, Sk), jnp.float32),
            pltpu.VMEM((4, M, 128), jnp.float32),
            pltpu.VMEM((4, M, D), jnp.float32),
            pltpu.VMEM((4, M, 128), jnp.float32),
            pltpu.SemaphoreType.DMA((4,)),
            pltpu.SemaphoreType.DMA((4,)),
            pltpu.SemaphoreType.DMA((4,)),
            pltpu.SemaphoreType.DMA((4,)),
        ],
        compiler_params=pltpu.CompilerParams(
            vmem_limit_bytes=100 * 1024 * 1024,
            disable_bounds_checks=True,
        ),
    )(q3, k3, v3)
    return out.reshape(B, Hq, Sq, D)
```
